```python
import jax
import jax.numpy as jnp

def _softmax(x, axis=-1):
    return jax.nn.softmax(x, axis=axis)
def _gelu(x):
    return jax.nn.gelu(x, approximate=True)
def _silu(x):
    return jax.nn.silu(x)
def _sigmoid(x):
    return jax.nn.sigmoid(x)
def _layernorm(x, axis=-1, eps=1e-5):
    m = jnp.mean(x, axis=axis, keepdims=True)
    v = jnp.var(x, axis=axis, keepdims=True)
    return (x - m) / jnp.sqrt(v + eps)
def _scatter_add(tgt, idx, src, axis=0):
    return tgt.at[idx].add(src)
def _segment_sum(src, seg, n):
    return jax.ops.segment_sum(src, seg, n)
class _Rng:
    def __init__(self, key):
        self._k = key
    def _next(self):
        self._k, sub = jax.random.split(self._k)
        return sub
    def normal(self, shape):
        return jax.random.normal(self._next(), shape, dtype=jnp.bfloat16)
    def randint(self, lo, hi, shape):
        return jax.random.randint(self._next(), shape, lo, hi, dtype=jnp.int32)
    def uniform(self, shape, lo=0.0, hi=1.0):
        return jax.random.uniform(self._next(), shape, jnp.bfloat16, lo, hi)
    def permutation(self, n):
        return jax.random.permutation(self._next(), n)


kernel_name = 'interleave_layers__sliding_block_cached__glu_gated_glu__decode'

def setup_inputs():
    _rng = _Rng(jax.random.key(int.from_bytes(__import__("os").urandom(4), "little")))
    _w = (lambda a: (lambda t: t.astype(jnp.bfloat16) if jnp.issubdtype(t.dtype, jnp.floating) else t)(jnp.asarray(a)))
    def _A_setup():
        B, Sq, D = 1, 1, 640
        Hq, Hkv, Sk, Dh = 32, 32, 32768, 192
        assert Hq % Hkv == 0, (Hq, Hkv)
        return {
            "x": _w((lambda *s: _rng.normal(s) * 0.05)(B, Sq, D)),
            "k_cache": _w((lambda *s: _rng.normal(s) * 0.05)(B, Hkv, Sk, Dh)),
            "v_cache": _w((lambda *s: _rng.normal(s) * 0.05)(B, Hkv, Sk, Dh)),
            "wq": _w((lambda *s: _rng.normal(s) * 0.05)(D, Hq * Dh) * (D ** -0.5)),
            "wo": _w((lambda *s: _rng.normal(s) * 0.05)(Hq * Dh, D) * ((Hq * Dh) ** -0.5)),
        }
    _A_in = _A_setup()

    def _B_setup():
        B, S, D, F = 1, 1, 640, 1536
        return {
            "x": _w((lambda *s: _rng.normal(s) * 0.05)(B, S, D)),
            "w_gate": _w((lambda *s: _rng.normal(s) * 0.05)(D, F)),
            "w_up": _w((lambda *s: _rng.normal(s) * 0.05)(D, F)),
            "w_down": _w((lambda *s: _rng.normal(s) * 0.05)(F, D)),
        }
    _B_in = _B_setup()

    return {
        "A_x": _A_in["x"],
        "A_k_cache": _A_in["k_cache"],
        "A_v_cache": _A_in["v_cache"],
        "A_wq": _A_in["wq"],
        "A_wo": _A_in["wo"],
        "B_x": _B_in["x"],
        "B_w_gate": _B_in["w_gate"],
        "B_w_up": _B_in["w_up"],
        "B_w_down": _B_in["w_down"],
    }

def reference(A_x, A_k_cache, A_v_cache, A_wq, A_wo, B_x, B_w_gate, B_w_up, B_w_down):
    def _A_ref(x, k_cache, v_cache, wq, wo):
        B, Sq, D = x.shape
        Hq, Dh = 32, 192
        Hkv, Sk = k_cache.shape[1], k_cache.shape[2]
        W = min(4096, max(256, Sk // 4))
        rep = Hq // Hkv
        q = (lambda x, *d: x.transpose(*d))((x @ wq).reshape(B, Sq, Hq, Dh), 0, 2, 1, 3)
        k = jnp.repeat(k_cache[:, :, Sk - W:, :], rep, axis=1)
        v = jnp.repeat(v_cache[:, :, Sk - W:, :], rep, axis=1)
        scores = jnp.einsum("bhqd,bhkd->bhqk", q, k) * (Dh ** -0.5)
        p = _softmax(scores, axis=-1)
        o = jnp.einsum("bhqk,bhkd->bhqd", p, v)
        return (lambda x, *d: x.transpose(*d))(o, 0, 2, 1, 3).reshape(B, Sq, Hq * Dh) @ wo

    def _B_ref(x, w_gate, w_up, w_down):
        g = jnp.einsum("bsd,df->bsf", x, w_gate)
        u = jnp.einsum("bsd,df->bsf", x, w_up)
        h = _sigmoid(g) * u
        return jnp.einsum("bsf,fd->bsd", h, w_down)

    x = A_x
    x = x + _A_ref(_layernorm(x, axis=-1), A_k_cache, A_v_cache, A_wq, A_wo)
    x = x + _B_ref(_layernorm(x, axis=-1), B_w_gate, B_w_up, B_w_down)
    x = x + _A_ref(_layernorm(x, axis=-1), A_k_cache, A_v_cache, A_wq, A_wo)
    x = x + _B_ref(_layernorm(x, axis=-1), B_w_gate, B_w_up, B_w_down)
    return x
```

```python
import functools
import jax
import jax.numpy as jnp
from jax import lax
import jax.experimental.pallas as pl
import jax.experimental.pallas.tpu as pltpu

BF = jnp.bfloat16
F32 = jnp.float32
U32 = jnp.uint32

D, H, DH, SK, W, F = 640, 32, 192, 32768, 4096, 1536
G = H // 2
PM = 2 * DH // 16
NJ = W // 128
ND = D // 128
NF = F // 128
EPS = 1e-5
SCALE = DH ** -0.5


def _tiles(a, lead):
    r, c = a.shape[-2:]
    n = len(lead)
    a = a.reshape(*lead, -1, 2, 8, c // 128, 128)
    return a.transpose(*range(n + 2), n + 3, n + 2, n + 4)


def _rows(w):
    return pltpu.bitcast(w.reshape(w.shape[0] * 8, 128), BF)


def _dot(a, b):
    return jnp.dot(a, b, preferred_element_type=F32)


def _dot_nt(a, b):
    return lax.dot_general(a, b, (((1,), (1,)), ((), ())), preferred_element_type=F32)


def _bf(x):
    return x.astype(BF).astype(F32)


def _layernorm(x):
    m = jnp.mean(x, axis=-1, keepdims=True)
    c = x - m
    v = jnp.mean(c * c, axis=-1, keepdims=True)
    return c / jnp.sqrt(v + EPS)


def _seq(*gens):
    for g in gens:
        yield from g


def _scaled(gen, k):
    for c in gen:
        yield c * k


def _run(*gens):
    clock = {i: 0.0 for i in range(len(gens))}
    while clock:
        i = min(clock, key=lambda k: (clock[k], k))
        c = next(gens[i], None)
        if c is None:
            del clock[i]
        else:
            clock[i] += c


def make(Y=2, YL=12, LAG=10, ST=500, FG=(360, 40, 140), FN=0, CP=7, FL=1, FV=1, STL=360, TAIL=60, name="decode", dma=True, layers=2, flags=None):
    def kernel(x_hbm, k_hbm, v_hbm, wq_hbm, wo_hbm, wg_hbm, wu_hbm, wd_hbm, o_ref,
               x_buf, k_buf, v_buf, wq_buf, wo_buf, wg_buf, wu_buf, wd_buf,
               x_s, xn_s, q_s, lhs_s, p_s, pb_s, l_s, a_s, b_s, o_s, acc_s, idx_s, sems):
        pending = []
        ties = {}

        def halves(src, dst, sem):
            return [pltpu.make_async_copy(src.at[:, a], dst.at[:, :, pl.ds(8 * a, 8)], sem) for a in range(2)]

        def kv_copies(src, dst, g, sem):
            return halves(src.at[g, :, :, pl.ds((SK - W) // 128, NJ)], dst.at[pl.ds(g * PM, PM)], sem)

        def group(t):
            sem = sems.at[t % 2]
            return (kv_copies(k_hbm, k_buf, t + 1, sem) + kv_copies(v_hbm, v_buf, t, sem)
                    + halves(wo_hbm.at[t], wo_buf.at[t], sem))

        first = ([pltpu.make_async_copy(x_hbm, x_buf, sems.at[2])] + halves(wq_hbm, wq_buf, sems.at[2])
                 + kv_copies(k_hbm, k_buf, 0, sems.at[2]))
        last = (kv_copies(v_hbm, v_buf, G - 1, sems.at[(G - 1) % 2])
                + halves(wo_hbm.at[G - 1], wo_buf.at[G - 1], sems.at[(G - 1) % 2]))
        gate_up = halves(wg_hbm, wg_buf, sems.at[G % 2]) + halves(wu_hbm, wu_buf, sems.at[G % 2])
        WD0 = 80
        down0 = halves(wd_hbm.at[pl.ds(0, WD0)], wd_buf.at[pl.ds(0, WD0)], sems.at[2])
        down1 = halves(wd_hbm.at[pl.ds(WD0, 96 - WD0)], wd_buf.at[pl.ds(WD0, 96 - WD0)], sems.at[3])

        def start(cs):
            if dma:
                for c in cs:
                    c.start()

        def wait(cs):
            if dma:
                for c in cs:
                    c.wait()

        start(first)
        start(group(0))
        for m in range(PM):
            idx_s[m] = 0

        ku, vu = k_buf.bitcast(U32), v_buf.bitcast(U32)
        wqu, wou = wq_buf.bitcast(U32), wo_buf.bitcast(U32)
        wgu, wuu, wdu = wg_buf.bitcast(U32), wu_buf.bitcast(U32), wd_buf.bitcast(U32)

        row = lax.broadcasted_iota(jnp.int32, (8, 128), 0)
        lane = lax.broadcasted_iota(jnp.int32, (8, 128), 1)
        head_of = [jnp.zeros_like(lane), (lane >= DH - 128).astype(jnp.int32), jnp.ones_like(lane)]

        def tile(ref, g, b, j):
            return _rows(ref[pl.ds(g * PM + 8 * b, 8), j])

        def chain(pairs, dot, cost, done):
            acc = [None]

            def add(r):
                acc[0] = r if acc[0] is None else acc[0] + r
                ties[id(acc)] = acc[0]

            n = len(pairs)
            for i, (lhs, rhs) in enumerate(pairs):
                r = dot(lhs(), rhs())
                pending.append(functools.partial(add, r))
                if i == n - 1:
                    pending.append(lambda: done(acc[0]))
                while len(pending) > LAG:
                    pending.pop(0)()
                yield cost

        def flush():
            while pending:
                pending.pop(0)()
            yield 0

        def q_proj(g):
            for b in range(3):
                def done(r, b=b):
                    q_s[g % 2, b] = _bf(r)
                yield from chain([(lambda k=k: xn_s[:, 128 * k:128 * (k + 1)],
                                   lambda k=k: _rows(wqu[8 * k:8 * k + 8, 3 * g + b])) for k in range(ND)], _dot, 8, done)

        def scores(g, s):
            for c in range(4):
                for b in range(3):
                    lhs_s[c, b] = jnp.where(row == 2 * c + head_of[b], q_s[g % 2, b], 0.0)
            for J in range(NJ // 4):
                yield from chain([(lambda c=c, b=b: lhs_s[c, b], lambda c=c, b=b: tile(ku, g, b, 4 * J + c))
                                  for c in range(4) for b in range(3)], _dot, 8, s.append)

        def pair_reduce(x, op):
            x = op(x, pltpu.roll(x, 4, 0))
            return op(x, pltpu.roll(x, 2, 0))

        def softmax(g, s, gap):
            while len(s) < NJ // 4:
                yield 4
            m = functools.reduce(jnp.maximum, s)
            m = jnp.max(pair_reduce(m, jnp.maximum), axis=1, keepdims=True)
            p = [jnp.exp((x - m) * SCALE) for x in s]
            l = functools.reduce(jnp.add, p)
            yield gap
            for J in range(NJ // 4):
                p_s[J] = p[J]
            l_s[g % 2] = l

        def values(g, y, steps):
            n = NJ - y
            always = (row + idx_s[0]) >= 0
            always = jnp.concatenate([always, always], axis=0)
            acc = None
            count, hist, links = 0, [], 0
            ties.clear()
            for m in range(PM):
                hh = m // (PM // 2)
                base = idx_s[m]
                cnt = (steps * (m + 1)) // PM - (steps * m) // PM
                ends = {(n * (k + 1)) // cnt - 1 for k in range(cnt)}
                prev, acc, part = acc, None, None
                for j in range(n):
                    if m % (PM // 2) == 0:
                        r = 2 * (j % 4) + hh
                        p = jnp.broadcast_to(p_s[j // 4, r:r + 1], (8, 128))
                        pb_s[j] = p
                    else:
                        p = pb_s[base + j]
                    t = pltpu.bitcast(vu[g * PM + m, j], BF).astype(F32) * jnp.concatenate([p, p], axis=0)
                    part = t if part is None else part + t
                    if j in ends:
                        if acc is None:
                            acc = part if prev is None else jnp.where(always, part, prev)
                        else:
                            acc = acc + part
                        part = None
                        links += 1
                        if CP and links % CP == 0 and j < n - 1:
                            lo, hi = acc[:8], acc[8:]
                            k = (links // CP) % 4
                            if k == 0:
                                lo = jnp.where(always[:8], lo, hi)
                            if k == 2:
                                hi = jnp.where(always[:8], hi, lo)
                            if k % 2 and ties:
                                for val in ties.values():
                                    lo = jnp.where(always[:8], lo, val)
                                ties.clear()
                            acc = jnp.concatenate([lo, hi], axis=0)
                    count += 1
                    if FN and count % FN == 0 and acc is not None:
                        hist.append(acc)
                        if len(hist) > FL:
                            old = hist.pop(0)
                            pb_s[idx_s[0] + NJ] = old[:8]
                            if FV:
                                vu[idx_s[0] + G * PM, 0] = pltpu.bitcast(old[8:], U32)
                    yield 1.5
                a_s[16 * m:16 * (m + 1)] = acc

        def values_mxu(g, y):
            for b in range(3):
                def done(r, b=b):
                    b_s[b] = jnp.where(row % 2 == head_of[b], r, 0.0)
                if y == 0:
                    b_s[b] = jnp.zeros((8, 128), F32)
                    continue
                yield from chain([(lambda j=j: jnp.where(row // 2 == j % 4, p_s[j // 4], 0.0),
                                   lambda j=j: tile(vu, g, b, j)) for j in range(NJ - y, NJ)], _dot_nt, 16, done)

        def finish(g, gap):
            l = jnp.sum(pair_reduce(l_s[g % 2], jnp.add), axis=1, keepdims=True)
            inv = jnp.broadcast_to(1.0 / l, (8, 128))
            inv = [jnp.broadcast_to(inv[hh:hh + 1], (8, 128)) for hh in range(2)]
            o = []
            for b in range(3):
                t = a_s[128 * b:128 * (b + 1)].T
                t = t.reshape(16, 8, 128).sum(axis=0) + b_s[b]
                t = jnp.broadcast_to(jnp.sum(t, axis=0, keepdims=True), (8, 128))
                o.append(_bf(t * jnp.where(head_of[b] == 0, inv[0], inv[1])))
                o_s[b] = o[b]
            for b, d in enumerate(gap):
                yield d
                ties[b] = o[b]

        def out_proj(g):
            for n in range(ND):
                def done(r, n=n):
                    acc_s[:, 128 * n:128 * (n + 1)] += r
                yield from chain([(lambda b=b: o_s[b], lambda b=b: _rows(wou[g, 8 * b:8 * b + 8, n])) for b in range(3)], _dot, 8, done)

        def layer(li, carry):
            loading = li == 0

            @pl.when(loading)
            def _():
                wait(first)
                start(group(1))
                x_s[...] = jnp.broadcast_to(x_buf[...].astype(F32), (8, D))

            x = x_s[...]
            acc_s[...] = x
            xn_s[...] = _bf(_layernorm(x))
            s = []
            _run(_seq(q_proj(0), flush(), q_proj(1), scores(0, s), flush()))
            _run(softmax(0, s, 0))
            a_s[...] = jnp.zeros(a_s.shape, F32)
            b_s[...] = jnp.zeros(b_s.shape, F32)
            l_s[1] = jnp.ones(l_s.shape[1:], F32)

            def step(t, c):
                @pl.when(loading)
                def _():
                    wait(group(t))

                    @pl.when(t + 2 < G - 1)
                    def _():
                        start(group(t + 2))

                    @pl.when(t + 2 == G - 1)
                    def _():
                        start(last)

                    @pl.when(t + 2 == G)
                    def _():
                        start(gate_up)

                s = []
                tm = 8 * (96 + 30) + 48 * Y
                tv = 36 * (NJ - Y)
                _run(finish(t + 1, FG), _seq(scores(t + 1, s), values_mxu(t, Y), out_proj(jnp.maximum(t - 1, 0)),
                          q_proj(jnp.minimum(t + 2, G - 1)), flush()),
                     _scaled(values(t, Y, ST), (tm + TAIL) / tv),
                     softmax(t + 1, s, 1000))
                return c

            lax.fori_loop(0, G - 1, step, 0)

            @pl.when(loading)
            def _():
                wait(last)
                start(down0)
                start(down1)

            _run(finish(G - 2, FG), _seq(values_mxu(G - 1, YL), out_proj(G - 2), flush()), values(G - 1, YL, STL))
            _run(_seq(finish(G - 1, FG), out_proj(G - 1), flush()))
            x = acc_s[...]
            xn_s[...] = _bf(_layernorm(x))

            @pl.when(loading)
            def _():
                wait(gate_up)

            xn = xn_s[...]
            hs = []
            for n in range(NF):
                gt = _dot(xn, _rows(wgu[:, n]))
                up = _dot(xn, _rows(wuu[:, n]))
                hs.append(_bf(up / (1.0 + jnp.exp(-gt))))
            h = jnp.concatenate(hs, axis=1)

            @pl.when(loading)
            def _():
                wait(down0)

            for n in range(ND):
                acc_s[:, 128 * n:128 * (n + 1)] += _dot(h[:, :16 * WD0], _rows(wdu[0:WD0, n]))

            @pl.when(loading)
            def _():
                wait(down1)

            for n in range(ND):
                x_s[:, 128 * n:128 * (n + 1)] = acc_s[:, 128 * n:128 * (n + 1)] + _dot(h[:, 16 * WD0:], _rows(wdu[WD0:, n]))
            return carry

        lax.fori_loop(0, layers, layer, 0)
        o_ref[...] = x_s[0:1, :].astype(BF)

    @jax.jit
    def fn(A_x, A_k_cache, A_v_cache, A_wq, A_wo, B_x, B_w_gate, B_w_up, B_w_down):
        del B_x
        kt = _tiles(jnp.transpose(A_k_cache, (0, 1, 3, 2)), (G,))
        vt = _tiles(jnp.transpose(A_v_cache, (0, 1, 3, 2)), (G,))
        hbm = pl.BlockSpec(memory_space=pltpu.HBM)
        out = pl.pallas_call(
            kernel,
            out_shape=jax.ShapeDtypeStruct((1, D), BF),
            in_specs=[hbm] * 8,
            scratch_shapes=[
                pltpu.VMEM((1, D), BF),
                pltpu.VMEM((G * PM, NJ, 16, 128), BF),
                pltpu.VMEM((G * PM + 1, NJ, 16, 128), BF),
                pltpu.VMEM((D // 16, H * DH // 128, 16, 128), BF),
                pltpu.VMEM((G, PM, ND, 16, 128), BF),
                pltpu.VMEM((D // 16, NF, 16, 128), BF),
                pltpu.VMEM((D // 16, NF, 16, 128), BF),
                pltpu.VMEM((F // 16, ND, 16, 128), BF),
                pltpu.VMEM((8, D), F32),
                pltpu.VMEM((8, D), F32),
                pltpu.VMEM((2, 3, 8, 128), F32),
                pltpu.VMEM((4, 3, 8, 128), F32),
                pltpu.VMEM((NJ // 4, 8, 128), F32),
                pltpu.VMEM((NJ + 1, 8, 128), F32),
                pltpu.VMEM((2, 8, 128), F32),
                pltpu.VMEM((2 * DH, 128), F32),
                pltpu.VMEM((3, 8, 128), F32),
                pltpu.VMEM((3, 8, 128), F32),
                pltpu.VMEM((8, D), F32),
                pltpu.SMEM((PM,), jnp.int32),
                pltpu.SemaphoreType.DMA((4,)),
            ],
            compiler_params=pltpu.CompilerParams(vmem_limit_bytes=127 * 1024 * 1024, flags=flags),
            name=name,
        )(A_x.reshape(1, D), kt, vt, _tiles(A_wq, ()), _tiles(A_wo, (G,)),
          _tiles(B_w_gate, ()), _tiles(B_w_up, ()), _tiles(B_w_down, ()))
        return out.reshape(1, 1, D)
    return fn


pallas_interleave_layers__sliding_block_cached__glu_gated_glu__decode_kernel = make()
```

```python
import functools

import jax
import jax.numpy as jnp
from jax import lax
import jax.experimental.pallas as pl
import jax.experimental.pallas.tpu as pltpu

BF16 = jnp.bfloat16
F32 = jnp.float32
U32 = jnp.uint32

D, H, DH, SK, F = 640, 32, 192, 32768, 1536
W = min(4096, max(256, SK // 4))
G = H // 2
PM = 2 * DH // 16
NJ = W // 128
ND = D // 128
NF = F // 128
LAYERS = 2
EPS = 1e-5
SCALE = DH ** -0.5

FIRST, TRIP, LAST = 2, 4, 2
TRIPS = (G - FIRST - LAST) // TRIP
MXU_BLOCKS = (6,) + (4,) * (G - 3) + (7, 22)
TUNING = ((3, 0.7, 1.66, 8, 500), (1, 0.72, 1.64, 6, 500), (2, 0.72, 1.62, 6, 320))
DOWN_SPLIT = 80
IN_FLIGHT = 3


def _tiles(a, lead=()):
    n = len(lead)
    a = a.reshape(*lead, -1, 2, 8, a.shape[-1] // 128, 128)
    return a.transpose(*range(n + 2), n + 3, n + 2, n + 4)


def _rows(w):
    return pltpu.bitcast(w.reshape(w.shape[0] * 8, 128), BF16)


def _dot(a, b):
    return jnp.dot(a, b, preferred_element_type=F32)


def _round(x):
    return x.astype(BF16).astype(F32)


def _layernorm(x):
    c = x - jnp.mean(x, axis=-1, keepdims=True)
    v = jnp.mean(c * c, axis=-1, keepdims=True)
    return _round(c), jnp.broadcast_to(1.0 / jnp.sqrt(v + EPS), (8, 128))


def _same_head(x, op):
    x = op(x, pltpu.roll(x, 4, 0))
    return op(x, pltpu.roll(x, 2, 0))


def _seq(steps):
    for step in steps:
        yield from step


def _interleave(*streams):
    clock = {i: 0.0 for i in range(len(streams))}
    while clock:
        i = min(clock, key=lambda k: (clock[k], k))
        cost = next(streams[i], None)
        if cost is None:
            del clock[i]
        else:
            clock[i] += cost
            assert clock[i] < 1e6, "streams wait for each other"


def _kernel(x_hbm, k_hbm, v_hbm, wq_hbm, wo_hbm, wg_hbm, wu_hbm, wd_hbm, out_ref,
            x_buf, k_buf, v_buf, wq_buf, wo_buf, wg_buf, wu_buf, wd_buf,
            x_s, xn_s, rs_s, q_s, lhs_s, p_s, pb_s, l_s, a_s, b_s, o_s, acc_s, zero_s, sems):

    def halves(src, dst, sem):
        return [pltpu.make_async_copy(src.at[:, a], dst.at[:, :, pl.ds(8 * a, 8)], sem) for a in range(2)]

    def window(src, dst, g, sem):
        return halves(src.at[g, :, :, pl.ds((SK - W) // 128, NJ)], dst.at[pl.ds(g * PM, PM)], sem)

    def pair_copies(t, with_k=True):
        sem = sems.at[t % IN_FLIGHT]
        return ((window(k_hbm, k_buf, t + 1, sem) if with_k else [])
                + window(v_hbm, v_buf, t, sem) + halves(wo_hbm.at[t], wo_buf.at[t], sem))

    def copies(i):
        sem = sems.at[i % IN_FLIGHT]
        if i < 0:
            return (halves(wq_hbm, wq_buf, sem) + window(k_hbm, k_buf, 0, sem)
                    + [pltpu.make_async_copy(x_hbm, x_buf, sem)])
        if i < G:
            return pair_copies(i, i < G - 1)
        if i == G:
            return halves(wg_hbm, wg_buf, sem) + halves(wu_hbm, wu_buf, sem)
        rows = pl.ds(0, DOWN_SPLIT) if i == G + 1 else pl.ds(DOWN_SPLIT, F // 16 - DOWN_SPLIT)
        return halves(wd_hbm.at[rows], wd_buf.at[rows], sem)

    def start(cs):
        for c in cs:
            c.start()

    def wait(cs):
        for c in cs:
            c.wait()

    for i in range(-1, IN_FLIGHT - 1):
        start(copies(i))
    for m in range(PM):
        zero_s[m] = 0

    ku, vu, wqu, wou, wgu, wuu, wdu = (
        r.bitcast(U32) for r in (k_buf, v_buf, wq_buf, wo_buf, wg_buf, wu_buf, wd_buf))

    row = lax.broadcasted_iota(jnp.int32, (8, 128), 0)
    lane = lax.broadcasted_iota(jnp.int32, (8, 128), 1)
    head_of = [jnp.zeros_like(lane), (lane >= DH - 128).astype(jnp.int32), jnp.ones_like(lane)]

    def tile(ref, g, b, j):
        return _rows(ref[pl.ds(g * PM + 8 * b, 8), j])

    def transpose_values(g, blocks):
        def body(j, carry):
            for b in range(3):
                vu[pl.ds(g * PM + 8 * b, 8), j] = pltpu.bitcast(tile(vu, g, b, j).T, U32).reshape(8, 8, 128)
            return carry
        lax.fori_loop(NJ - blocks, NJ, body, 0)

    def advance(i):
        wait(copies(i))
        if i + IN_FLIGHT <= G + 2:
            start(copies(i + IN_FLIGHT))
        if 0 <= i < G:
            transpose_values(i, MXU_BLOCKS[i])

    def block(first, count, shift):
        end = first + count
        final = end == G
        lag, links_per_reg, reg_cost, mark_every, finish_time = TUNING[2 if final else 1 if first else 0]
        pending, due, done, scores_of = [], {}, set(), {}
        chain_state = dict(acc=None, links=0, sums=0)
        for t in range(-2, first):
            done.update([("values", t), ("mxu_values", t), ("finish", t - 1), ("out", t - 1)])
        done.update([("softmax", first), ("q", first + 1)] if first else [("finish", -1), ("out", -1)])
        always = (row + zero_s[0]) >= 0

        def need(*keys):
            while not done.issuperset(keys):
                yield 2

        def mxu_need(*keys):
            while not done.issuperset(keys):
                if pending:
                    pending.pop(0)()
                yield 8

        def mxu_sum(operands, then):
            chain_state["sums"] += 1
            name = ("sum", chain_state["sums"])
            acc = [None]

            def add(r, last):
                acc[0] = r if acc[0] is None else acc[0] + r
                due[name] = acc[0]
                if last:
                    then(acc[0])

            for i, (lhs, rhs) in enumerate(operands):
                pending.append(functools.partial(add, _dot(lhs(), rhs()), i == len(operands) - 1))
                while len(pending) > lag:
                    pending.pop(0)()
                yield 8

        def mxu_drain():
            while pending:
                pending.pop(0)()
                yield 8

        def q_proj(t):
            for b in range(3):
                def then(r, b=b):
                    q_s[t % 2, b] = _round(r * rs_s[0])
                    if b == 2:
                        done.add(("q", t))
                yield from mxu_sum(
                    [(lambda k=k: xn_s[:, 128 * k:128 * (k + 1)],
                      lambda k=k: _rows(wqu[8 * k:8 * k + 8, 3 * (t + shift) + b])) for k in range(ND)], then)

        def scores(t):
            yield from mxu_need(("q", t))
            for c in range(4):
                for b in range(3):
                    lhs_s[t % 2, c, b] = jnp.where(row == 2 * c + head_of[b], q_s[t % 2, b], 0.0)
            for J in range(NJ // 4):
                yield from mxu_sum(
                    [(lambda c=c, b=b: lhs_s[t % 2, c, b], lambda c=c, b=b: tile(ku, t + shift, b, 4 * J + c))
                     for c in range(4) for b in range(3)], scores_of.setdefault(t, []).append)

        def softmax(t):
            s = scores_of.setdefault(t, [])
            while len(s) < NJ // 4:
                yield 2
            yield from need(("values", t - 2), ("mxu_values", t - 2), ("finish", t - 2))
            m = functools.reduce(jnp.maximum, s)
            m = jnp.max(_same_head(m, jnp.maximum), axis=1, keepdims=True)
            p = [jnp.exp((x - m) * SCALE) for x in s]
            for J in range(NJ // 4):
                p_s[t % 2, J] = p[J]
            l_s[t % 2] = functools.reduce(jnp.add, p)
            done.add(("softmax", t))

        def values(t):
            yield from need(("softmax", t), ("finish", t - 2))
            n = NJ - MXU_BLOCKS[t]
            links = int(links_per_reg * n * PM)
            always2 = jnp.concatenate([always, always], axis=0)
            for m in range(PM):
                h = m // (PM // 2)
                slot = zero_s[m] + h
                here = (links * (m + 1)) // PM - (links * m) // PM
                ends = {(n * (k + 1)) // here - 1 for k in range(here)}
                prev, acc, part = chain_state["acc"], None, None
                for j in range(n):
                    if m % (PM // 2) == 0:
                        r = 2 * (j % 4) + h
                        p = jnp.broadcast_to(p_s[t % 2, j // 4, r:r + 1], (8, 128))
                        pb_s[h, j] = p
                    else:
                        p = pb_s[slot, j]
                    v = pltpu.bitcast(vu[(t + shift) * PM + m, j], BF16).astype(F32)
                    v = v * jnp.concatenate([p, p], axis=0)
                    part = v if part is None else part + v
                    if j in ends:
                        if acc is None:
                            acc = part if prev is None else jnp.where(always2, part, prev)
                        else:
                            acc = acc + part
                        part = None
                        chain_state["links"] += 1
                        if chain_state["links"] % mark_every == 0 and j < n - 1:
                            lo, hi = acc[:8], acc[8:]
                            phase = (chain_state["links"] // mark_every) % 4
                            if phase == 0:
                                lo = jnp.where(always, lo, hi)
                            elif phase == 2:
                                hi = jnp.where(always, hi, lo)
                            else:
                                for other in due.values():
                                    lo = jnp.where(always, lo, other)
                                due.clear()
                            acc = jnp.concatenate([lo, hi], axis=0)
                    yield reg_cost
                a_s[t % 2, 16 * m:16 * (m + 1)] = acc
                chain_state["acc"] = acc
            done.add(("values", t))

        def mxu_values(t):
            yield from mxu_need(("softmax", t), ("finish", t - 2))
            for b in range(3):
                def then(r, b=b):
                    b_s[t % 2, b] = jnp.where(row % 2 == head_of[b], r, 0.0)
                    if b == 2:
                        done.add(("mxu_values", t))
                yield from mxu_sum(
                    [(lambda j=j: jnp.where(row // 2 == j % 4, p_s[t % 2, j // 4], 0.0),
                      lambda j=j: tile(vu, t + shift, b, j)) for j in range(NJ - MXU_BLOCKS[t], NJ)], then)

        def finish(t):
            yield from need(("values", t), ("mxu_values", t), ("out", t - 2))
            l = jnp.sum(_same_head(l_s[t % 2], jnp.add), axis=1, keepdims=True)
            inv = jnp.broadcast_to(1.0 / l, (8, 128))
            inv = [jnp.broadcast_to(inv[h:h + 1], (8, 128)) for h in range(2)]
            o = []
            for b in range(3):
                a = a_s[t % 2, 128 * b:128 * (b + 1)].T
                a = a.reshape(16, 8, 128).sum(axis=0) + b_s[t % 2, b]
                a = jnp.broadcast_to(jnp.sum(a, axis=0, keepdims=True), (8, 128))
                o.append(_round(a * jnp.where(head_of[b] == 0, inv[0], inv[1])))
                o_s[t % 2, b] = o[b]
            done.add(("finish", t))
            for b, delay in enumerate((finish_time, 40, 140)):
                yield delay
                due["o", b] = o[b]

        def out_proj(t):
            yield from mxu_need(("finish", t))
            for k in range(ND):
                def then(r, k=k):
                    acc_s[:, 128 * k:128 * (k + 1)] += r
                yield from mxu_sum(
                    [(lambda b=b: o_s[t % 2, b], lambda b=b: _rows(wou[t + shift, 8 * b:8 * b + 8, k]))
                     for b in range(3)], then)
            done.add(("out", t))

        mxu = [] if first else [q_proj(0), q_proj(1), scores(0)]
        for t in range(first, end):
            mxu += [scores(t + 1)] if t + 1 < G else []
            mxu += [q_proj(t + 2)] if t + 2 < G else []
            mxu += [mxu_values(t)] + ([out_proj(t - 1)] if 0 < t < G - 1 else [])
        mxu += [out_proj(G - 2), out_proj(G - 1)] if final else []
        _interleave(
            _seq(mxu + [mxu_drain()]),
            _seq([finish(t) for t in range(max(first - 1, 0), end if final else end - 1)]),
            _seq([values(t) for t in range(first, end)]),
            _seq([softmax(t) for t in range(first + 1 if first else 0, min(end + 1, G))]))

    def glu(loading):
        x = acc_s[:, :D]
        xn, rs = _layernorm(x)
        if loading:
            advance(G)
        hidden = []
        for n in range(NF):
            gate = _dot(xn, _rows(wgu[:, n])) * rs
            up = _dot(xn, _rows(wuu[:, n])) * rs
            hidden.append(_round(up / (1.0 + jnp.exp(-gate))))
        out = [x[:, 128 * n:128 * (n + 1)] for n in range(ND)]
        for k in range(NF):
            if loading and 8 * k in (0, DOWN_SPLIT):
                advance(G + 1 + (k > 0))
            out = [out[n] + _dot(hidden[k], _rows(wdu[8 * k:8 * k + 8, n])) for n in range(ND)]
        x_s[:, :D] = jnp.concatenate(out, axis=1)

    def layer(index, carry):
        loading = index == 0

        @pl.when(loading)
        def _():
            for i in range(-1, FIRST):
                advance(i)
            x_s[:, :D] = jnp.broadcast_to(x_buf[...].astype(F32), (8, D))

        x = x_s[:, :D]
        acc_s[:, :D] = x
        xn_s[:, :D], rs_s[0] = _layernorm(x)
        block(0, FIRST, 0)

        def trip(it, carry):
            @pl.when(loading)
            def _():
                for i in range(FIRST, FIRST + TRIP):
                    t = i + it * TRIP
                    wait(pair_copies(t))
                    for late in range(G - 1, G - LAST + IN_FLIGHT):
                        if (late - IN_FLIGHT - i) % TRIP == 0:
                            pl.when(t + IN_FLIGHT == late)(lambda late=late: start(copies(late)))
                    pl.when(t + IN_FLIGHT < G - 1)(lambda t=t: start(pair_copies(t + IN_FLIGHT)))
                    transpose_values(t, MXU_BLOCKS[i])

            block(FIRST, TRIP, it * TRIP)
            return carry

        lax.fori_loop(0, TRIPS, trip, 0)

        @pl.when(loading)
        def _():
            for i in range(G - LAST, G):
                advance(i)

        block(G - LAST, LAST, 0)
        pl.when(loading)(lambda: glu(True))
        pl.when(jnp.logical_not(loading))(lambda: glu(False))
        return carry

    lax.fori_loop(0, LAYERS, layer, 0)
    out_ref[...] = x_s[0:1, :D].astype(BF16)


@jax.jit
def pallas_interleave_layers__sliding_block_cached__glu_gated_glu__decode_kernel(
    A_x: jax.Array,
    A_k_cache: jax.Array,
    A_v_cache: jax.Array,
    A_wq: jax.Array,
    A_wo: jax.Array,
    B_x: jax.Array,
    B_w_gate: jax.Array,
    B_w_up: jax.Array,
    B_w_down: jax.Array,
):
    del B_x
    assert A_x.shape == (1, 1, D) and A_k_cache.shape == A_v_cache.shape == (1, H, SK, DH)
    operands = (
        A_x.reshape(1, D),
        _tiles(jnp.transpose(A_k_cache, (0, 1, 3, 2)), (G,)),
        _tiles(jnp.transpose(A_v_cache, (0, 1, 3, 2)), (G,)),
        _tiles(A_wq),
        _tiles(A_wo, (G,)),
        _tiles(B_w_gate),
        _tiles(B_w_up),
        _tiles(B_w_down),
    )
    out = pl.pallas_call(
        _kernel,
        out_shape=jax.ShapeDtypeStruct((1, D), BF16),
        in_specs=[pl.BlockSpec(memory_space=pltpu.HBM)] * len(operands),
        scratch_shapes=[
            pltpu.VMEM((1, D), BF16),
            pltpu.VMEM((G * PM, NJ, 16, 128), BF16),
            pltpu.VMEM((G * PM, NJ, 16, 128), BF16),
            pltpu.VMEM((D // 16, H * DH // 128, 16, 128), BF16),
            pltpu.VMEM((G, PM, ND, 16, 128), BF16),
            pltpu.VMEM((D // 16, NF, 16, 128), BF16),
            pltpu.VMEM((D // 16, NF, 16, 128), BF16),
            pltpu.VMEM((F // 16, ND, 16, 128), BF16),
            pltpu.VMEM((8, 1024), F32),
            pltpu.VMEM((8, 1024), F32),
            pltpu.VMEM((4, 8, 128), F32),
            pltpu.VMEM((2, 4, 8, 128), F32),
            pltpu.VMEM((2, 4, 3, 8, 128), F32),
            pltpu.VMEM((2, NJ // 4, 8, 128), F32),
            pltpu.VMEM((2, NJ, 8, 128), F32),
            pltpu.VMEM((4, 8, 128), F32),
            pltpu.VMEM((2, 2 * DH, 128), F32),
            pltpu.VMEM((2, 4, 8, 128), F32),
            pltpu.VMEM((2, 4, 8, 128), F32),
            pltpu.VMEM((8, 1024), F32),
            pltpu.SMEM((PM,), jnp.int32),
            pltpu.SemaphoreType.DMA((IN_FLIGHT,)),
        ],
        compiler_params=pltpu.CompilerParams(vmem_limit_bytes=127 * 1024 * 1024),
        name="decode_layers",
    )(*operands)
    return out.reshape(1, 1, D)
```

```python
import functools

import jax
import jax.numpy as jnp
from jax import lax
import jax.experimental.pallas as pl
import jax.experimental.pallas.tpu as pltpu

BF16 = jnp.bfloat16
F32 = jnp.float32
U32 = jnp.uint32

D, H, DH, SK, F = 640, 32, 192, 32768, 1536
W = min(4096, max(256, SK // 4))
G = H // 2
PM = 2 * DH // 16
NJ = W // 128
ND = D // 128
NF = F // 128
LAYERS = 2
EPS = 1e-5
SCALE = DH ** -0.5

FIRST, TRIP, LAST = 2, 4, 2
TRIPS = (G - FIRST - LAST) // TRIP
MXU_BLOCKS = (5,) + (3,) * (G - 3) + (6, 21)
WIDE = tuple(range(2, 26, 4))
TUNING = ((1, 0.68, 1.56, 6, 320), (1, 0.66, 1.58, 6, 320), (1, 0.68, 1.56, 6, 420))
DOWN_SPLIT = 80
IN_FLIGHT = 3


def _tiles(a, lead=()):
    n = len(lead)
    a = a.reshape(*lead, -1, 2, 8, a.shape[-1] // 128, 128)
    return a.transpose(*range(n + 2), n + 3, n + 2, n + 4)


def _rows(w):
    return pltpu.bitcast(w.reshape(w.shape[0] * 8, 128), BF16)


def _dot(a, b):
    return jnp.dot(a, b, preferred_element_type=F32)


def _round(x):
    return x.astype(BF16).astype(F32)


def _layernorm(x):
    c = x - jnp.mean(x, axis=-1, keepdims=True)
    v = jnp.mean(c * c, axis=-1, keepdims=True)
    return _round(c), jnp.broadcast_to(1.0 / jnp.sqrt(v + EPS), (8, 128))


def _same_head(x, op):
    x = op(x, pltpu.roll(x, 4, 0))
    return op(x, pltpu.roll(x, 2, 0))


def _seq(steps):
    for step in steps:
        yield from step


def _interleave(*streams):
    clock = {i: 0.0 for i in range(len(streams))}
    while clock:
        i = min(clock, key=lambda k: (clock[k], k))
        cost = next(streams[i], None)
        if cost is None:
            del clock[i]
        else:
            clock[i] += cost
            assert clock[i] < 1e6, "streams wait for each other"


def _kernel(x_hbm, k_hbm, v_hbm, wq_hbm, wo_hbm, wg_hbm, wu_hbm, wd_hbm, out_ref,
            x_buf, k_buf, v_buf, wq_buf, wo_buf, wg_buf, wu_buf, wd_buf,
            wide_buf, x_s, xn_s, rs_s, q_s, lhs_s, p_s, pb_s, l_s, a_s, b_s, o_s, acc_s, zero_s, sems):

    def halves(src, dst, sem):
        return [pltpu.make_async_copy(src.at[:, a], dst.at[:, :, pl.ds(8 * a, 8)], sem) for a in range(2)]

    def window(src, dst, g, sem):
        return halves(src.at[g, :, :, pl.ds((SK - W) // 128, NJ)], dst.at[pl.ds(g * PM, PM)], sem)

    def pair_copies(t, with_k=True):
        sem = sems.at[t % IN_FLIGHT]
        return ((window(k_hbm, k_buf, t + 1, sem) if with_k else [])
                + window(v_hbm, v_buf, t, sem) + halves(wo_hbm.at[t], wo_buf.at[t], sem))

    def copies(i):
        sem = sems.at[i % IN_FLIGHT]
        if i < 0:
            return (halves(wq_hbm, wq_buf, sem) + window(k_hbm, k_buf, 0, sem)
                    + [pltpu.make_async_copy(x_hbm, x_buf, sem)])
        if i < G:
            return pair_copies(i, i < G - 1)
        if i == G:
            return halves(wg_hbm, wg_buf, sem) + halves(wu_hbm, wu_buf, sem)
        rows = pl.ds(0, DOWN_SPLIT) if i == G + 1 else pl.ds(DOWN_SPLIT, F // 16 - DOWN_SPLIT)
        return halves(wd_hbm.at[rows], wd_buf.at[rows], sem)

    def start(cs):
        for c in cs:
            c.start()

    def wait(cs):
        for c in cs:
            c.wait()

    for i in range(-1, IN_FLIGHT - 1):
        start(copies(i))
    for m in range(PM):
        zero_s[m] = 0

    ku, vu, wqu, wou, wgu, wuu, wdu = (
        r.bitcast(U32) for r in (k_buf, v_buf, wq_buf, wo_buf, wg_buf, wu_buf, wd_buf))

    row = lax.broadcasted_iota(jnp.int32, (8, 128), 0)
    lane = lax.broadcasted_iota(jnp.int32, (8, 128), 1)
    head_of = [jnp.zeros_like(lane), (lane >= DH - 128).astype(jnp.int32), jnp.ones_like(lane)]

    def tile(ref, g, b, j):
        return _rows(ref[pl.ds(g * PM + 8 * b, 8), j])

    def prepare_values(g, mxu_blocks):
        def transpose(j, carry):
            for b in range(3):
                vu[pl.ds(g * PM + 8 * b, 8), j] = pltpu.bitcast(tile(vu, g, b, j).T, U32).reshape(8, 8, 128)
            return carry

        def widen(m, carry):
            for k, j in enumerate(WIDE):
                if j < NJ - mxu_blocks:
                    v = pltpu.bitcast(vu[g * PM + m, j], BF16).astype(F32)
                    vu[g * PM + m, j] = pltpu.bitcast(v[:8], U32)
                    wide_buf[g, m, k] = v[8:]
            return carry

        lax.fori_loop(NJ - mxu_blocks, NJ, transpose, 0)
        lax.fori_loop(0, PM, widen, 0)

    def advance(i):
        wait(copies(i))
        if i + IN_FLIGHT <= G + 2:
            start(copies(i + IN_FLIGHT))
        if 0 <= i < G:
            prepare_values(i, MXU_BLOCKS[i])

    def block(first, count, shift):
        end = first + count
        final = end == G
        lag, links_per_reg, reg_cost, mark_every, finish_time = TUNING[2 if final else 1 if first else 0]
        pending, due, done, scores_of = [], {}, set(), {}
        chain_state = dict(acc=None, links=0, sums=0)
        for t in range(-2, first):
            done.update([("values", t), ("mxu_values", t), ("finish", t - 1), ("out", t - 1)])
        done.update([("softmax", first), ("q", first + 1)] if first else [("finish", -1), ("out", -1)])
        always = (row + zero_s[0]) >= 0

        def need(*keys):
            while not done.issuperset(keys):
                yield 2

        def mxu_need(*keys):
            while not done.issuperset(keys):
                if pending:
                    pending.pop(0)()
                yield 8

        def mxu_sum(operands, then):
            chain_state["sums"] += 1
            name = ("sum", chain_state["sums"])
            acc = [None]

            def add(r, last):
                acc[0] = r if acc[0] is None else acc[0] + r
                due[name] = acc[0]
                if last:
                    then(acc[0])

            for i, (lhs, rhs) in enumerate(operands):
                pending.append(functools.partial(add, _dot(lhs(), rhs()), i == len(operands) - 1))
                while len(pending) > lag:
                    pending.pop(0)()
                yield 8

        def mxu_drain():
            while pending:
                pending.pop(0)()
                yield 8

        def q_proj(t):
            for b in range(3):
                def then(r, b=b):
                    q_s[t % 2, b] = _round(r * rs_s[0])
                    if b == 2:
                        done.add(("q", t))
                yield from mxu_sum(
                    [(lambda k=k: xn_s[:, 128 * k:128 * (k + 1)],
                      lambda k=k: _rows(wqu[8 * k:8 * k + 8, 3 * (t + shift) + b])) for k in range(ND)], then)

        def scores(t):
            yield from mxu_need(("q", t))
            for c in range(4):
                for b in range(3):
                    lhs_s[t % 2, c, b] = jnp.where(row == 2 * c + head_of[b], q_s[t % 2, b], 0.0)
            for J in range(NJ // 4):
                yield from mxu_sum(
                    [(lambda c=c, b=b: lhs_s[t % 2, c, b], lambda c=c, b=b: tile(ku, t + shift, b, 4 * J + c))
                     for c in range(4) for b in range(3)], scores_of.setdefault(t, []).append)

        def softmax(t):
            s = scores_of.setdefault(t, [])
            while len(s) < NJ // 4:
                yield 2
            yield from need(("values", t - 2), ("mxu_values", t - 2), ("finish", t - 2))
            m = functools.reduce(jnp.maximum, s)
            m = jnp.max(_same_head(m, jnp.maximum), axis=1, keepdims=True)
            p = [jnp.exp((x - m) * SCALE) for x in s]
            for J in range(NJ // 4):
                p_s[t % 2, J] = p[J]
            l_s[t % 2] = functools.reduce(jnp.add, p)
            done.add(("softmax", t))

        def values(t):
            yield from need(("softmax", t), ("finish", t - 2))
            n = NJ - MXU_BLOCKS[t]
            links = int(links_per_reg * n * PM)
            always2 = jnp.concatenate([always, always], axis=0)
            for m in range(PM):
                h = m // (PM // 2)
                slot = zero_s[m] + h
                here = (links * (m + 1)) // PM - (links * m) // PM
                ends = {(n * (k + 1)) // here - 1 for k in range(here)}
                prev, acc, part = chain_state["acc"], None, None
                for j in range(n):
                    if m % (PM // 2) == 0:
                        r = 2 * (j % 4) + h
                        p = jnp.broadcast_to(p_s[t % 2, j // 4, r:r + 1], (8, 128))
                        pb_s[h, j] = p
                    else:
                        p = pb_s[slot, j]
                    v = vu[(t + shift) * PM + m, j]
                    if j in WIDE:
                        v = jnp.concatenate([pltpu.bitcast(v, F32), wide_buf[t + shift, m, WIDE.index(j)]], axis=0)
                    else:
                        v = pltpu.bitcast(v, BF16).astype(F32)
                    v = v * jnp.concatenate([p, p], axis=0)
                    part = v if part is None else part + v
                    if j in ends:
                        if acc is None:
                            acc = part if prev is None else jnp.where(always2, part, prev)
                        else:
                            acc = acc + part
                        part = None
                        chain_state["links"] += 1
                        if chain_state["links"] % mark_every == 0 and j < n - 1:
                            lo, hi = acc[:8], acc[8:]
                            phase = (chain_state["links"] // mark_every) % 4
                            if phase == 0:
                                lo = jnp.where(always, lo, hi)
                            elif phase == 2:
                                hi = jnp.where(always, hi, lo)
                            else:
                                for other in due.values():
                                    lo = jnp.where(always, lo, other)
                                due.clear()
                            acc = jnp.concatenate([lo, hi], axis=0)
                    yield reg_cost
                a_s[t % 2, 16 * m:16 * (m + 1)] = acc
                chain_state["acc"] = acc
            done.add(("values", t))

        def mxu_values(t):
            yield from mxu_need(("softmax", t), ("finish", t - 2))
            for b in range(3):
                def then(r, b=b):
                    b_s[t % 2, b] = jnp.where(row % 2 == head_of[b], r, 0.0)
                    if b == 2:
                        done.add(("mxu_values", t))
                yield from mxu_sum(
                    [(lambda j=j: jnp.where(row // 2 == j % 4, p_s[t % 2, j // 4], 0.0),
                      lambda j=j: tile(vu, t + shift, b, j)) for j in range(NJ - MXU_BLOCKS[t], NJ)], then)

        def finish(t):
            yield from need(("values", t), ("mxu_values", t), ("out", t - 2))
            l = jnp.sum(_same_head(l_s[t % 2], jnp.add), axis=1, keepdims=True)
            inv = jnp.broadcast_to(1.0 / l, (8, 128))
            inv = [jnp.broadcast_to(inv[h:h + 1], (8, 128)) for h in range(2)]
            o = []
            for b in range(3):
                a = a_s[t % 2, 128 * b:128 * (b + 1)].T
                a = a.reshape(16, 8, 128).sum(axis=0) + b_s[t % 2, b]
                a = jnp.broadcast_to(jnp.sum(a, axis=0, keepdims=True), (8, 128))
                o.append(_round(a * jnp.where(head_of[b] == 0, inv[0], inv[1])))
                o_s[t % 2, b] = o[b]
            done.add(("finish", t))
            for b, delay in enumerate((finish_time, 40, 140)):
                yield delay
                due["o", b] = o[b]

        def out_proj(t):
            yield from mxu_need(("finish", t))
            for k in range(ND):
                def then(r, k=k):
                    acc_s[:, 128 * k:128 * (k + 1)] += r
                yield from mxu_sum(
                    [(lambda b=b: o_s[t % 2, b], lambda b=b: _rows(wou[t + shift, 8 * b:8 * b + 8, k]))
                     for b in range(3)], then)
            done.add(("out", t))

        mxu = [] if first else [q_proj(0), q_proj(1), scores(0)]
        for t in range(first, end):
            mxu += [scores(t + 1)] if t + 1 < G else []
            mxu += [q_proj(t + 2)] if t + 2 < G else []
            mxu += [mxu_values(t)] + ([out_proj(t - 1)] if 0 < t < G - 1 else [])
        mxu += [out_proj(G - 2), out_proj(G - 1)] if final else []
        _interleave(
            _seq(mxu + [mxu_drain()]),
            _seq([finish(t) for t in range(max(first - 1, 0), end if final else end - 1)]),
            _seq([values(t) for t in range(first, end)]),
            _seq([softmax(t) for t in range(first + 1 if first else 0, min(end + 1, G))]))

    def glu(loading):
        x = acc_s[:, :D]
        xn, rs = _layernorm(x)
        if loading:
            advance(G)
        hidden = []
        for n in range(NF):
            gate = _dot(xn, _rows(wgu[:, n])) * rs
            up = _dot(xn, _rows(wuu[:, n])) * rs
            hidden.append(_round(up / (1.0 + jnp.exp(-gate))))
        out = [x[:, 128 * n:128 * (n + 1)] for n in range(ND)]
        for k in range(NF):
            if loading and 8 * k in (0, DOWN_SPLIT):
                advance(G + 1 + (k > 0))
            out = [out[n] + _dot(hidden[k], _rows(wdu[8 * k:8 * k + 8, n])) for n in range(ND)]
        x_s[:, :D] = jnp.concatenate(out, axis=1)

    def layer(index, carry):
        loading = index == 0

        @pl.when(loading)
        def _():
            for i in range(-1, FIRST):
                advance(i)
            x_s[:, :D] = jnp.broadcast_to(x_buf[...].astype(F32), (8, D))

        x = x_s[:, :D]
        acc_s[:, :D] = x
        xn_s[:, :D], rs_s[0] = _layernorm(x)
        block(0, FIRST, 0)

        def trip(it, carry):
            @pl.when(loading)
            def _():
                for i in range(FIRST, FIRST + TRIP):
                    t = i + it * TRIP
                    wait(pair_copies(t))
                    for late in range(G - 1, G - LAST + IN_FLIGHT):
                        if (late - IN_FLIGHT - i) % TRIP == 0:
                            pl.when(t + IN_FLIGHT == late)(lambda late=late: start(copies(late)))
                    pl.when(t + IN_FLIGHT < G - 1)(lambda t=t: start(pair_copies(t + IN_FLIGHT)))
                    prepare_values(t, MXU_BLOCKS[i])

            block(FIRST, TRIP, it * TRIP)
            return carry

        lax.fori_loop(0, TRIPS, trip, 0)

        @pl.when(loading)
        def _():
            for i in range(G - LAST, G):
                advance(i)

        block(G - LAST, LAST, 0)
        pl.when(loading)(lambda: glu(True))
        pl.when(jnp.logical_not(loading))(lambda: glu(False))
        return carry

    lax.fori_loop(0, LAYERS, layer, 0)
    out_ref[...] = x_s[0:1, :D].astype(BF16)


@jax.jit
def pallas_interleave_layers__sliding_block_cached__glu_gated_glu__decode_kernel(
    A_x: jax.Array,
    A_k_cache: jax.Array,
    A_v_cache: jax.Array,
    A_wq: jax.Array,
    A_wo: jax.Array,
    B_x: jax.Array,
    B_w_gate: jax.Array,
    B_w_up: jax.Array,
    B_w_down: jax.Array,
):
    del B_x
    assert A_x.shape == (1, 1, D) and A_k_cache.shape == A_v_cache.shape == (1, H, SK, DH)
    operands = (
        A_x.reshape(1, D),
        _tiles(jnp.transpose(A_k_cache, (0, 1, 3, 2)), (G,)),
        _tiles(jnp.transpose(A_v_cache, (0, 1, 3, 2)), (G,)),
        _tiles(A_wq),
        _tiles(A_wo, (G,)),
        _tiles(B_w_gate),
        _tiles(B_w_up),
        _tiles(B_w_down),
    )
    out = pl.pallas_call(
        _kernel,
        out_shape=jax.ShapeDtypeStruct((1, D), BF16),
        in_specs=[pl.BlockSpec(memory_space=pltpu.HBM)] * len(operands),
        scratch_shapes=[
            pltpu.VMEM((1, D), BF16),
            pltpu.VMEM((G * PM, NJ, 16, 128), BF16),
            pltpu.VMEM((G * PM, NJ, 16, 128), BF16),
            pltpu.VMEM((D // 16, H * DH // 128, 16, 128), BF16),
            pltpu.VMEM((G, PM, ND, 16, 128), BF16),
            pltpu.VMEM((D // 16, NF, 16, 128), BF16),
            pltpu.VMEM((D // 16, NF, 16, 128), BF16),
            pltpu.VMEM((F // 16, ND, 16, 128), BF16),
            pltpu.VMEM((G, PM, len(WIDE), 8, 128), F32),
            pltpu.VMEM((8, 1024), F32),
            pltpu.VMEM((8, 1024), F32),
            pltpu.VMEM((4, 8, 128), F32),
            pltpu.VMEM((2, 4, 8, 128), F32),
            pltpu.VMEM((2, 4, 3, 8, 128), F32),
            pltpu.VMEM((2, NJ // 4, 8, 128), F32),
            pltpu.VMEM((2, NJ, 8, 128), F32),
            pltpu.VMEM((4, 8, 128), F32),
            pltpu.VMEM((2, 2 * DH, 128), F32),
            pltpu.VMEM((2, 4, 8, 128), F32),
            pltpu.VMEM((2, 4, 8, 128), F32),
            pltpu.VMEM((8, 1024), F32),
            pltpu.SMEM((PM,), jnp.int32),
            pltpu.SemaphoreType.DMA((IN_FLIGHT,)),
        ],
        compiler_params=pltpu.CompilerParams(vmem_limit_bytes=127 * 1024 * 1024),
        name="decode_layers",
    )(*operands)
    return out.reshape(1, 1, D)
```

```python
import functools

import jax
import jax.numpy as jnp
from jax import lax
import jax.experimental.pallas as pl
import jax.experimental.pallas.tpu as pltpu

BF16 = jnp.bfloat16
F32 = jnp.float32
U32 = jnp.uint32

D, H, DH, SK, F = 640, 32, 192, 32768, 1536
W = min(4096, max(256, SK // 4))
G = H // 2
PM = 2 * DH // 16
NJ = W // 128
ND = D // 128
NF = F // 128
LAYERS = 2
EPS = 1e-5
SCALE = DH ** -0.5

FIRST, TRIP, LAST = 2, 4, 2
TRIPS = (G - FIRST - LAST) // TRIP
MXU_BLOCKS = (5,) + (3,) * (G - 3) + (6, 21)
WIDE = tuple(range(2, 26, 4))
TUNING = ((2, 0.68, 1.56, 6, 320), (2, 0.64, 1.56, 6, 420), (2, 0.68, 1.52, 7, 320))
DOWN_SPLIT = 80
IN_FLIGHT = 3


def _tiles(a, lead=()):
    n = len(lead)
    a = a.reshape(*lead, -1, 2, 8, a.shape[-1] // 128, 128)
    return a.transpose(*range(n + 2), n + 3, n + 2, n + 4)


def _rows(w):
    return pltpu.bitcast(w.reshape(w.shape[0] * 8, 128), BF16)


def _dot(a, b):
    return jnp.dot(a, b, preferred_element_type=F32)


def _round(x):
    return x.astype(BF16).astype(F32)


def _layernorm(x):
    c = x - jnp.mean(x, axis=-1, keepdims=True)
    v = jnp.mean(c * c, axis=-1, keepdims=True)
    return _round(c), jnp.broadcast_to(1.0 / jnp.sqrt(v + EPS), (8, 128))


def _same_head(x, op):
    x = op(x, pltpu.roll(x, 4, 0))
    return op(x, pltpu.roll(x, 2, 0))


def _seq(steps):
    for step in steps:
        yield from step


def _interleave(*streams):
    clock = {i: 0.0 for i in range(len(streams))}
    while clock:
        i = min(clock, key=lambda k: (clock[k], k))
        cost = next(streams[i], None)
        if cost is None:
            del clock[i]
        else:
            clock[i] += cost
            assert clock[i] < 1e6, "streams wait for each other"


def _kernel(x_hbm, k_hbm, v_hbm, wq_hbm, wo_hbm, wg_hbm, wu_hbm, wd_hbm, out_ref,
            x_buf, k_buf, v_buf, wq_buf, wo_buf, wg_buf, wu_buf, wd_buf,
            wide_buf, x_s, xn_s, rs_s, q_s, lhs_s, p_s, pb_s, l_s, a_s, b_s, o_s, acc_s, zero_s, sems):

    def halves(src, dst, sem):
        return [pltpu.make_async_copy(src.at[:, a], dst.at[:, :, pl.ds(8 * a, 8)], sem) for a in range(2)]

    def window(src, dst, g, sem):
        return halves(src.at[g, :, :, pl.ds((SK - W) // 128, NJ)], dst.at[pl.ds(g * PM, PM)], sem)

    def pair_copies(t, with_k=True):
        sem = sems.at[t % IN_FLIGHT]
        return ((window(k_hbm, k_buf, t + 1, sem) if with_k else [])
                + window(v_hbm, v_buf, t, sem) + halves(wo_hbm.at[t], wo_buf.at[t], sem))

    def copies(i):
        sem = sems.at[i % IN_FLIGHT]
        if i < 0:
            return (halves(wq_hbm, wq_buf, sem) + window(k_hbm, k_buf, 0, sem)
                    + [pltpu.make_async_copy(x_hbm, x_buf, sem)])
        if i < G:
            return pair_copies(i, i < G - 1)
        if i == G:
            return halves(wg_hbm, wg_buf, sem) + halves(wu_hbm, wu_buf, sem)
        rows = pl.ds(0, DOWN_SPLIT) if i == G + 1 else pl.ds(DOWN_SPLIT, F // 16 - DOWN_SPLIT)
        return halves(wd_hbm.at[rows], wd_buf.at[rows], sem)

    def start(cs):
        for c in cs:
            c.start()

    def wait(cs):
        for c in cs:
            c.wait()

    for i in range(-1, IN_FLIGHT - 1):
        start(copies(i))
    for m in range(PM):
        zero_s[m] = 0

    ku, vu, wqu, wou, wgu, wuu, wdu = (
        r.bitcast(U32) for r in (k_buf, v_buf, wq_buf, wo_buf, wg_buf, wu_buf, wd_buf))

    row = lax.broadcasted_iota(jnp.int32, (8, 128), 0)
    lane = lax.broadcasted_iota(jnp.int32, (8, 128), 1)
    head_of = [jnp.zeros_like(lane), (lane >= DH - 128).astype(jnp.int32), jnp.ones_like(lane)]

    def tile(ref, g, b, j):
        return _rows(ref[pl.ds(g * PM + 8 * b, 8), j])

    def prepare_values(g, mxu_blocks):
        def transpose(j, carry):
            for b in range(3):
                vu[pl.ds(g * PM + 8 * b, 8), j] = pltpu.bitcast(tile(vu, g, b, j).T, U32).reshape(8, 8, 128)
            return carry

        def widen(m, carry):
            for k, j in enumerate(WIDE):
                if j < NJ - mxu_blocks:
                    v = pltpu.bitcast(vu[g * PM + m, j], BF16).astype(F32)
                    vu[g * PM + m, j] = pltpu.bitcast(v[:8], U32)
                    wide_buf[g, m, k] = v[8:]
            return carry

        lax.fori_loop(NJ - mxu_blocks, NJ, transpose, 0)
        lax.fori_loop(0, PM, widen, 0)

    def advance(i):
        wait(copies(i))
        if i + IN_FLIGHT <= G + 2:
            start(copies(i + IN_FLIGHT))
        if 0 <= i < G:
            prepare_values(i, MXU_BLOCKS[i])

    def block(first, count, shift):
        end = first + count
        final = end == G
        lag, links_per_reg, reg_cost, mark_every, finish_time = TUNING[2 if final else 1 if first else 0]
        pending, due, done, scores_of = [], {}, set(), {}
        chain_state = dict(acc=None, links=0, sums=0)
        for t in range(-2, first):
            done.update([("values", t), ("mxu_values", t), ("finish", t - 1), ("out", t - 1)])
        done.update([("softmax", first), ("q", first + 1)] if first else [("finish", -1), ("out", -1)])
        always = (row + zero_s[0]) >= 0

        def need(*keys):
            while not done.issuperset(keys):
                yield 2

        def mxu_need(*keys):
            while not done.issuperset(keys):
                if pending:
                    pending.pop(0)()
                yield 8

        def mxu_sum(operands, then):
            chain_state["sums"] += 1
            name = ("sum", chain_state["sums"])
            acc = [None]

            def add(r, last):
                acc[0] = r if acc[0] is None else acc[0] + r
                due[name] = acc[0]
                if last:
                    then(acc[0])

            for i, (lhs, rhs) in enumerate(operands):
                pending.append(functools.partial(add, _dot(lhs(), rhs()), i == len(operands) - 1))
                while len(pending) > lag:
                    pending.pop(0)()
                yield 8

        def mxu_drain():
            while pending:
                pending.pop(0)()
                yield 8

        def q_proj(t):
            sums = []
            for b in range(3):
                def then(r, b=b):
                    q_s[t % 2, b] = _round(r * rs_s[0])
                    if b == 2:
                        done.add(("q", t))
                sums.append(mxu_sum(
                    [(lambda k=k: xn_s[:, 128 * k:128 * (k + 1)],
                      lambda k=k, b=b: _rows(wqu[8 * k:8 * k + 8, 3 * (t + shift) + b])) for k in range(ND)], then))
            for _ in range(ND):
                for one in sums:
                    yield next(one)

        def scores(t):
            yield from mxu_need(("q", t))
            for c in range(4):
                for b in range(3):
                    lhs_s[t % 2, c, b] = jnp.where(row == 2 * c + head_of[b], q_s[t % 2, b], 0.0)
            for J in range(NJ // 4):
                yield from mxu_sum(
                    [(lambda c=c, b=b: lhs_s[t % 2, c, b], lambda c=c, b=b: tile(ku, t + shift, b, 4 * J + c))
                     for b in range(3) for c in range(4)], scores_of.setdefault(t, []).append)

        def softmax(t):
            s = scores_of.setdefault(t, [])
            while len(s) < NJ // 4:
                yield 2
            yield from need(("values", t - 2), ("mxu_values", t - 2), ("finish", t - 2))
            m = functools.reduce(jnp.maximum, s)
            m = jnp.max(_same_head(m, jnp.maximum), axis=1, keepdims=True)
            p = [jnp.exp((x - m) * SCALE) for x in s]
            for J in range(NJ // 4):
                p_s[t % 2, J] = p[J]
            l_s[t % 2] = functools.reduce(jnp.add, p)
            done.add(("softmax", t))

        def values(t):
            yield from need(("softmax", t), ("finish", t - 2))
            n = NJ - MXU_BLOCKS[t]
            links = int(links_per_reg * n * PM)
            always2 = jnp.concatenate([always, always], axis=0)
            for m in range(PM):
                h = m // (PM // 2)
                slot = zero_s[m] + h
                here = (links * (m + 1)) // PM - (links * m) // PM
                ends = {(n * (k + 1)) // here - 1 for k in range(here)}
                prev, acc, part = chain_state["acc"], None, None
                for j in range(n):
                    if m % (PM // 2) == 0:
                        r = 2 * (j % 4) + h
                        p = jnp.broadcast_to(p_s[t % 2, j // 4, r:r + 1], (8, 128))
                        pb_s[h, j] = p
                    else:
                        p = pb_s[slot, j]
                    v = vu[(t + shift) * PM + m, j]
                    if j in WIDE:
                        v = jnp.concatenate([pltpu.bitcast(v, F32), wide_buf[t + shift, m, WIDE.index(j)]], axis=0)
                    else:
                        v = pltpu.bitcast(v, BF16).astype(F32)
                    v = v * jnp.concatenate([p, p], axis=0)
                    part = v if part is None else part + v
                    if j in ends:
                        if acc is None:
                            acc = part if prev is None else jnp.where(always2, part, prev)
                        else:
                            acc = acc + part
                        part = None
                        chain_state["links"] += 1
                        if chain_state["links"] % mark_every == 0 and j < n - 1:
                            lo, hi = acc[:8], acc[8:]
                            phase = (chain_state["links"] // mark_every) % 4
                            if phase == 0:
                                lo = jnp.where(always, lo, hi)
                            elif phase == 2:
                                hi = jnp.where(always, hi, lo)
                            else:
                                for other in due.values():
                                    lo = jnp.where(always, lo, other)
                                due.clear()
                            acc = jnp.concatenate([lo, hi], axis=0)
                    yield reg_cost
                a_s[t % 2, 16 * m:16 * (m + 1)] = acc
                chain_state["acc"] = acc
            done.add(("values", t))

        def mxu_values(t):
            yield from mxu_need(("softmax", t), ("finish", t - 2))
            for b in range(3):
                def then(r, b=b):
                    b_s[t % 2, b] = jnp.where(row % 2 == head_of[b], r, 0.0)
                    if b == 2:
                        done.add(("mxu_values", t))
                yield from mxu_sum(
                    [(lambda j=j: jnp.where(row // 2 == j % 4, p_s[t % 2, j // 4], 0.0),
                      lambda j=j: tile(vu, t + shift, b, j)) for j in range(NJ - MXU_BLOCKS[t], NJ)], then)

        def finish(t):
            yield from need(("values", t), ("mxu_values", t), ("out", t - 2))
            l = jnp.sum(_same_head(l_s[t % 2], jnp.add), axis=1, keepdims=True)
            inv = jnp.broadcast_to(1.0 / l, (8, 128))
            inv = [jnp.broadcast_to(inv[h:h + 1], (8, 128)) for h in range(2)]
            o = []
            for b in range(3):
                a = a_s[t % 2, 128 * b:128 * (b + 1)].T
                a = a.reshape(16, 8, 128).sum(axis=0) + b_s[t % 2, b]
                a = jnp.broadcast_to(jnp.sum(a, axis=0, keepdims=True), (8, 128))
                o.append(_round(a * jnp.where(head_of[b] == 0, inv[0], inv[1])))
                o_s[t % 2, b] = o[b]
            done.add(("finish", t))
            for b, delay in enumerate((finish_time, 40, 140)):
                yield delay
                due["o", b] = o[b]

        def out_proj(t):
            yield from mxu_need(("finish", t))
            for k in range(ND):
                def then(r, k=k):
                    acc_s[:, 128 * k:128 * (k + 1)] += r
                yield from mxu_sum(
                    [(lambda b=b: o_s[t % 2, b], lambda b=b: _rows(wou[t + shift, 8 * b:8 * b + 8, k]))
                     for b in range(3)], then)
            done.add(("out", t))

        mxu = [] if first else [q_proj(0), q_proj(1), scores(0)]
        for t in range(first, end):
            mxu += [scores(t + 1)] if t + 1 < G else []
            mxu += [q_proj(t + 2)] if t + 2 < G else []
            mxu += [mxu_values(t)] + ([out_proj(t - 1)] if 0 < t < G - 1 else [])
        mxu += [out_proj(G - 2), out_proj(G - 1)] if final else []
        _interleave(
            _seq(mxu + [mxu_drain()]),
            _seq([finish(t) for t in range(max(first - 1, 0), end if final else end - 1)]),
            _seq([values(t) for t in range(first, end)]),
            _seq([softmax(t) for t in range(first + 1 if first else 0, min(end + 1, G))]))

    def glu(loading):
        x = acc_s[:, :D]
        xn, rs = _layernorm(x)
        if loading:
            advance(G)
        hidden = []
        for n in range(NF):
            gate = _dot(xn, _rows(wgu[:, n])) * rs
            up = _dot(xn, _rows(wuu[:, n])) * rs
            hidden.append(_round(up / (1.0 + jnp.exp(-gate))))
        out = [x[:, 128 * n:128 * (n + 1)] for n in range(ND)]
        for k in range(NF):
            if loading and 8 * k in (0, DOWN_SPLIT):
                advance(G + 1 + (k > 0))
            out = [out[n] + _dot(hidden[k], _rows(wdu[8 * k:8 * k + 8, n])) for n in range(ND)]
        x_s[:, :D] = jnp.concatenate(out, axis=1)

    def layer(index, carry):
        loading = index == 0

        @pl.when(loading)
        def _():
            for i in range(-1, FIRST):
                advance(i)
            x_s[:, :D] = jnp.broadcast_to(x_buf[...].astype(F32), (8, D))

        x = x_s[:, :D]
        acc_s[:, :D] = x
        xn_s[:, :D], rs_s[0] = _layernorm(x)
        block(0, FIRST, 0)

        def trip(it, carry):
            @pl.when(loading)
            def _():
                for i in range(FIRST, FIRST + TRIP):
                    t = i + it * TRIP
                    wait(pair_copies(t))
                    for late in range(G - 1, G - LAST + IN_FLIGHT):
                        if (late - IN_FLIGHT - i) % TRIP == 0:
                            pl.when(t + IN_FLIGHT == late)(lambda late=late: start(copies(late)))
                    pl.when(t + IN_FLIGHT < G - 1)(lambda t=t: start(pair_copies(t + IN_FLIGHT)))
                    prepare_values(t, MXU_BLOCKS[i])

            block(FIRST, TRIP, it * TRIP)
            return carry

        lax.fori_loop(0, TRIPS, trip, 0)

        @pl.when(loading)
        def _():
            for i in range(G - LAST, G):
                advance(i)

        block(G - LAST, LAST, 0)
        pl.when(loading)(lambda: glu(True))
        pl.when(jnp.logical_not(loading))(lambda: glu(False))
        return carry

    lax.fori_loop(0, LAYERS, layer, 0)
    out_ref[...] = x_s[0:1, :D].astype(BF16)


@jax.jit
def pallas_interleave_layers__sliding_block_cached__glu_gated_glu__decode_kernel(
    A_x: jax.Array,
    A_k_cache: jax.Array,
    A_v_cache: jax.Array,
    A_wq: jax.Array,
    A_wo: jax.Array,
    B_x: jax.Array,
    B_w_gate: jax.Array,
    B_w_up: jax.Array,
    B_w_down: jax.Array,
):
    del B_x
    assert A_x.shape == (1, 1, D) and A_k_cache.shape == A_v_cache.shape == (1, H, SK, DH)
    operands = (
        A_x.reshape(1, D),
        _tiles(jnp.transpose(A_k_cache, (0, 1, 3, 2)), (G,)),
        _tiles(jnp.transpose(A_v_cache, (0, 1, 3, 2)), (G,)),
        _tiles(A_wq),
        _tiles(A_wo, (G,)),
        _tiles(B_w_gate),
        _tiles(B_w_up),
        _tiles(B_w_down),
    )
    out = pl.pallas_call(
        _kernel,
        out_shape=jax.ShapeDtypeStruct((1, D), BF16),
        in_specs=[pl.BlockSpec(memory_space=pltpu.HBM)] * len(operands),
        scratch_shapes=[
            pltpu.VMEM((1, D), BF16),
            pltpu.VMEM((G * PM, NJ, 16, 128), BF16),
            pltpu.VMEM((G * PM, NJ, 16, 128), BF16),
            pltpu.VMEM((D // 16, H * DH // 128, 16, 128), BF16),
            pltpu.VMEM((G, PM, ND, 16, 128), BF16),
            pltpu.VMEM((D // 16, NF, 16, 128), BF16),
            pltpu.VMEM((D // 16, NF, 16, 128), BF16),
            pltpu.VMEM((F // 16, ND, 16, 128), BF16),
            pltpu.VMEM((G, PM, len(WIDE), 8, 128), F32),
            pltpu.VMEM((8, 1024), F32),
            pltpu.VMEM((8, 1024), F32),
            pltpu.VMEM((4, 8, 128), F32),
            pltpu.VMEM((2, 4, 8, 128), F32),
            pltpu.VMEM((2, 4, 3, 8, 128), F32),
            pltpu.VMEM((2, NJ // 4, 8, 128), F32),
            pltpu.VMEM((2, NJ, 8, 128), F32),
            pltpu.VMEM((4, 8, 128), F32),
            pltpu.VMEM((2, 2 * DH, 128), F32),
            pltpu.VMEM((2, 4, 8, 128), F32),
            pltpu.VMEM((2, 4, 8, 128), F32),
            pltpu.VMEM((8, 1024), F32),
            pltpu.SMEM((PM,), jnp.int32),
            pltpu.SemaphoreType.DMA((IN_FLIGHT,)),
        ],
        compiler_params=pltpu.CompilerParams(vmem_limit_bytes=127 * 1024 * 1024),
        name="decode_layers",
    )(*operands)
    return out.reshape(1, 1, D)
```
